```python
import jax
import jax.numpy as jnp

def _softmax(x, axis=-1):
    return jax.nn.softmax(x, axis=axis)

def _gelu(x):
    return jax.nn.gelu(x, approximate=True)

def _silu(x):
    return jax.nn.silu(x)

def _sigmoid(x):
    return jax.nn.sigmoid(x)

def _layernorm(x, axis=-1, eps=1e-05):
    m = jnp.mean(x, axis=axis, keepdims=True)
    v = jnp.var(x, axis=axis, keepdims=True)
    return (x - m) / jnp.sqrt(v + eps)

def _scatter_add(tgt, idx, src, axis=0):
    return tgt.at[idx].add(src)

def _segment_sum(src, seg, n):
    return jax.ops.segment_sum(src, seg, n)

class _Rng:

    def __init__(self, key):
        self._k = key

    def _next(self):
        self._k, sub = jax.random.split(self._k)
        return sub

    def normal(self, shape):
        return jax.random.normal(self._next(), shape, dtype=jnp.bfloat16)

    def randint(self, lo, hi, shape):
        return jax.random.randint(self._next(), shape, lo, hi, dtype=jnp.int32)

    def uniform(self, shape, lo=0.0, hi=1.0):
        return jax.random.uniform(self._next(), shape, jnp.bfloat16, lo, hi)

    def permutation(self, n):
        return jax.random.permutation(self._next(), n)
kernel_name = 'interleave_layers__sliding_local_dilated__mixer_gmlp__prompt'

def setup_inputs():
    _rng = _Rng(jax.random.key(int.from_bytes(__import__("os").urandom(4), "little")))
    _w = lambda a: (lambda t: t.astype(jnp.bfloat16) if jnp.issubdtype(t.dtype, jnp.floating) else t)(jnp.asarray(a))

    def _A_setup():
        B, S, D = (1, 2048, 576)
        return {'x': _w((lambda *s: _rng.normal(s) * 0.05)(B, S, D)), 'wqkv': _w((lambda *s: _rng.normal(s) * 0.05)(D, 3 * D)), 'wo': _w((lambda *s: _rng.normal(s) * 0.05)(D, D))}
    _A_in = _A_setup()

    def _B_setup():
        B, S, D, F = (1, 2048, 576, 4608)
        Fh = F // 2
        return {'x': _w((lambda *s: _rng.normal(s) * 0.05)(B, S, D)), 'w_in': _w((lambda *s: _rng.normal(s) * 0.05)(D, 2 * Fh)), 'w_sp': _w(0.01 * (lambda *s: _rng.normal(s) * 0.05)(S, S)), 'b_sp': _w(1.0 + 0.01 * (lambda *s: _rng.normal(s) * 0.05)(S)), 'w_out': _w((lambda *s: _rng.normal(s) * 0.05)(Fh, D))}
    _B_in = _B_setup()
    return {'A_x': _A_in['x'], 'A_wqkv': _A_in['wqkv'], 'A_wo': _A_in['wo'], 'B_x': _B_in['x'], 'B_w_in': _B_in['w_in'], 'B_w_sp': _B_in['w_sp'], 'B_b_sp': _B_in['b_sp'], 'B_w_out': _B_in['w_out']}

def reference(A_x, A_wqkv, A_wo, B_x, B_w_in, B_w_sp, B_b_sp, B_w_out):

    def _A_ref(x, wqkv, wo):
        B, S, D = x.shape
        H = 32
        Dh = D // H
        W, dil = (8, 2)
        qkv = (lambda x, *d: x.transpose(*d))((x @ wqkv).reshape(B, S, 3, H, Dh), 2, 0, 3, 1, 4)
        q, k, v = (qkv[0], qkv[1], qkv[2])
        scale = Dh ** (-0.5)
        pos = jnp.arange(S)
        off = jnp.arange(W) * dil
        idx = pos[:, None] - off[None, :]
        mask = idx >= 0
        idx_c = jnp.where(mask, idx, 0).reshape(-1)
        kg = k[:, :, idx_c, :].reshape(B, H, S, W, Dh)
        vg = v[:, :, idx_c, :].reshape(B, H, S, W, Dh)
        logits = jnp.einsum('bhsd,bhswd->bhsw', q, kg) * scale
        logits = jnp.where(mask[None, None, :, :], logits, -1000000000.0)
        attn = _softmax(logits, axis=-1)
        o = jnp.einsum('bhsw,bhswd->bhsd', attn, vg)
        return (lambda x, *d: x.transpose(*d))(o, 0, 2, 1, 3).reshape(B, S, D) @ wo

    def _B_ref(x, w_in, w_sp, b_sp, w_out):
        B, S, D = x.shape
        F = w_in.shape[-1]
        Fh = F // 2
        z = _gelu(jnp.einsum('bsd,df->bsf', x, w_in))
        z1 = z[..., :Fh].copy()
        z2 = _layernorm(z[..., Fh:], axis=-1)
        g = jnp.einsum('ts,bsf->btf', w_sp, z2) + b_sp[None, :, None]
        return jnp.einsum('bsf,fd->bsd', z1 * g, w_out)
    x = A_x
    x = x + _A_ref(_layernorm(x, axis=-1), A_wqkv, A_wo)
    x = x + _B_ref(_layernorm(x, axis=-1), B_w_in, B_w_sp, B_b_sp, B_w_out)
    x = x + _A_ref(_layernorm(x, axis=-1), A_wqkv, A_wo)
    x = x + _B_ref(_layernorm(x, axis=-1), B_w_in, B_w_sp, B_b_sp, B_w_out)
    return x
```

```python
import math

import jax
import jax.numpy as jnp
import jax.experimental.pallas as pl
import jax.experimental.pallas.tpu as pltpu

S, D, H, DH, W, DIL = 2048, 576, 32, 18, 8, 2
FH = 2304
BM = 256
NB = S // BM
HALO = 16
CH = 576
LV = 1
CF = 576
YK = 1
NQ = 2 ** LV
FQ, BQ, SQ = FH // NQ, BM // NQ, S // NQ
NWC = min(NB, 6) if NB != 4 else 4
WC = 2 * FH // NWC
EPS = 1e-5
F32, BF16 = jnp.float32, jnp.bfloat16


def _dot(a, b):
    return jnp.dot(a, b, preferred_element_type=F32)


def _dot_nt(a, b):
    return jax.lax.dot_general(a, b, (((1,), (1,)), ((), ())), preferred_element_type=F32)


def _ln(x):
    m = jnp.mean(x, axis=0, keepdims=True)
    c = x - m
    v = jnp.mean(c * c, axis=0, keepdims=True)
    return c * jax.lax.rsqrt(v + EPS)


def _gelu(x):
    c0 = math.sqrt(2.0 / math.pi)
    u = x * (c0 + (c0 * 0.044715) * (x * x))
    hx = 0.5 * x
    return hx + hx * jnp.tanh(u)


def _strassen_side(blk, lv, left):
    if lv == 0:
        return [blk[0][0]]
    h = len(blk) // 2
    a11, a12, a21, a22 = (
        [row[c:c + h] for row in blk[r:r + h]] for r in (0, h) for c in (0, h))
    if left:
        ops = [_add(a11, a22), _add(a21, a22), a11, a22, _add(a11, a12),
               _sub(a21, a11), _sub(a12, a22)]
    else:
        ops = [_add(a11, a22), a11, _sub(a12, a22), _sub(a21, a11), a22,
               _add(a11, a12), _add(a21, a22)]
    return [o for m in ops for o in _strassen_side(m, lv - 1, left)]


def _strassen_out(ms, lv):
    if lv == 0:
        return [[ms[0]]]
    n = len(ms) // 7
    m1, m2, m3, m4, m5, m6, m7 = (
        _strassen_out(ms[k * n:(k + 1) * n], lv - 1) for k in range(7))
    c11 = _add(_sub(_add(m1, m4), m5), m7)
    c22 = _add(_add(_sub(m1, m2), m3), m6)
    top = [l + r for l, r in zip(c11, _add(m3, m5))]
    return top + [l + r for l, r in zip(_add(m2, m4), c22)]


def _add(a, b):
    return [[x + y for x, y in zip(r, t)] for r, t in zip(a, b)]


def _sub(a, b):
    return [[x - y for x, y in zip(r, t)] for r, t in zip(a, b)]


def _interleave(*gens):
    gens = list(gens)
    while gens:
        for g in list(gens):
            if next(g, _kernel) is _kernel:
                gens.remove(g)


def _kernel(x_hbm, wqkv_hbm, wo_hbm, win_hbm, wsp_hbm, b_hbm, wout_hbm, o_hbm,
            xin, wqkv_raw, wo_raw, T, wqkv, wo, win_raw, win, wsp, bsp, wout,
            X, Y, XN, Z2, K, V, Os, Zf, Hs, obuf, sems, wsem, osem):
    def win_copy(j):
        cols = pl.ds(pl.multiple_of(j * WC, 128), WC)
        return pltpu.make_async_copy(win_hbm.at[:, cols], win_raw.at[:, cols], wsem.at[j])

    cps = [
        pltpu.make_async_copy(wqkv_hbm, wqkv_raw, sems.at[0]),
        pltpu.make_async_copy(x_hbm, xin, sems.at[1]),
        pltpu.make_async_copy(wo_hbm, wo_raw, sems.at[2]),
        pltpu.make_async_copy(b_hbm, bsp, sems.at[3]),
        pltpu.make_async_copy(wout_hbm, wout, sems.at[4]),
        pltpu.make_async_copy(wsp_hbm, wsp, sems.at[5]),
    ]
    for c in cps[:3]:
        c.start()

    cps[0].wait()
    for j in range(5):
        n = min(128, D - j * 128)
        T[j, :, 0:n] = wqkv_raw[j * 128:j * 128 + n, :].astype(F32).T

    def gather(base, d, n):
        return [T[j, pl.ds(base + d, H, stride=DH), 0:n[j]] for j in range(5)]

    for part, dst in ((0, 0), (1, 640), (2, 1152)):
        for d in range(DH):
            r = dst + d * H if (part != 1 or d < 16) else 576 + (d - 16) * H
            wqkv[r:r + H, :] = jnp.concatenate(
                gather(part * D, d, (128, 128, 128, 128, 64)), axis=1).astype(BF16)
    wqkv[1728:1792, :] = jnp.zeros((64, D), BF16)
    cps[2].wait()
    for j in range(5):
        n = min(128, D - j * 128)
        T[j, 0:D, 0:n] = wo_raw[:, j * 128:j * 128 + n].astype(F32)
    for t in range(5):
        blk = [jnp.concatenate(gather(0, d, (128, 128, 128, 128, 64)), axis=1)
               if d < DH else jnp.zeros((H, D), F32) for d in range(4 * t, 4 * t + 4)]
        wo[:, t * 128:(t + 1) * 128] = jnp.concatenate(blk, axis=0).T.astype(BF16)
    cps[1].wait()
    for j in reversed(range(NWC)):
        win_copy(j).start()
    for c in cps[3:]:
        c.start()

    qscale = DH ** -0.5 * math.log2(math.e)
    lane = jax.lax.broadcasted_iota(jnp.int32, (BM, 128), 1)

    def zero_halo():
        K[:, 0:HALO, :] = jnp.zeros((5, HALO, 128), F32)
        V[:, 0:HALO, :] = jnp.zeros((5, HALO, 128), F32)

    def layer_a(x, i, cols):
        xn = _ln(x).T.astype(BF16)
        parts = []
        for n0, n1 in ((0, 640), (640, 1152), (1152, 1792)):
            yield
            parts.append(_dot_nt(xn, wqkv[n0:n1, :]))
        qkv = jnp.concatenate(parts, axis=1)
        yield
        t = qkv[:, 512:640]
        q = [qkv[:, j * 128:(j + 1) * 128] * qscale for j in range(4)]
        q.append(jnp.where(lane < 64, t * qscale, 0.0))
        for j in range(4):
            K[j, HALO:, :] = qkv[:, 640 + j * 128:768 + j * 128]
        K[4, HALO:, :] = pltpu.roll(t, 64, 1)
        for j in range(5):
            V[j, HALO:, :] = qkv[:, 1152 + j * 128:1280 + j * 128]
        R = 16
        for r0 in range(0, BM, R):
            lg = []
            for w in range(W):
                s = HALO + r0 - DIL * w
                a = q[0][r0:r0 + R] * K[0, s:s + R, :]
                for j in range(1, 5):
                    a = a + q[j][r0:r0 + R] * K[j, s:s + R, :]
                a = a + pltpu.roll(a, 64, 1)
                a = a + pltpu.roll(a, 32, 1)
                if r0 < DIL * w:
                    row = jax.lax.broadcasted_iota(jnp.int32, (R, 128), 0) + (i * BM + r0)
                    a = jnp.where(row >= DIL * w, a, -1e9)
                lg.append(a)
            m = lg[0]
            for w in range(1, W):
                m = jnp.maximum(m, lg[w])
            p = [jnp.exp2(a - m) for a in lg]
            den = p[0]
            for w in range(1, W):
                den = den + p[w]
            inv = 1.0 / den
            o = []
            for j in range(5):
                a = p[0] * V[j, HALO + r0:HALO + r0 + R, :]
                for w in range(1, W):
                    s = HALO + r0 - DIL * w
                    a = a + p[w] * V[j, s:s + R, :]
                o.append((a * inv).astype(BF16))
            Os[r0:r0 + R, :] = jnp.concatenate(o, axis=1)
            if (r0 + R) % (BM // 4) == 0:
                yield
        for j in range(5):
            K[j, 0:HALO, :] = K[j, BM:BM + HALO, :]
            V[j, 0:HALO, :] = V[j, BM:BM + HALO, :]
        X[:, cols] = x + _dot_nt(wo[...], Os[...])

    def cols_of(i):
        return pl.ds(pl.multiple_of(i * BM, BM), BM)

    def b_front(i, slot):
        cols = cols_of(i)
        xn = _ln(X[:, cols]).astype(BF16)
        XN[slot, :, cols] = xn
        for c0 in range(0, FH, CF):
            yield
            Zf[c0:c0 + CF, :] = _gelu(_dot(win[FH + c0:FH + c0 + CF, :], xn))

    def f_tail(i, slot):
        def total(f):
            acc = f(Zf[0:64, :])
            for r in range(64, FH, 64):
                acc = acc + f(Zf[r:r + 64, :])
            return jnp.sum(acc, axis=0, keepdims=True) * (1.0 / FH)
        m = total(lambda z: z)
        yield
        rs = jax.lax.rsqrt(total(lambda z: (z - m) * (z - m)) + EPS)
        sc = pl.ds(pl.multiple_of(i * BQ, BQ), BQ)
        for r0 in range(0, FQ, 32):
            if r0 % (FQ // 2) == 0:
                yield
            zs = [(Zf[r * FQ + r0:r * FQ + r0 + 32, :] - m) * rs for r in range(NQ)]
            blk = [[z[:, c * BQ:(c + 1) * BQ] for c in range(NQ)] for z in zs]
            for k, o in enumerate(_strassen_side(blk, LV, True)):
                Z2[slot, k, r0:r0 + 32, sc] = o.astype(BF16)

    def seq(*gens):
        for g in gens:
            yield from g

    def b_back(i, slot, store):
        cols = cols_of(i)
        xn = XN[slot, :, cols]
        x = X[:, cols]
        b = bsp[:, cols].astype(F32)
        blk = [[jnp.concatenate(
            [wsp[pl.ds(pl.multiple_of(i * BM + c * BQ, BQ), BQ),
                 n * BM + r * BQ:n * BM + (r + 1) * BQ] for n in range(NB)],
            axis=1).astype(F32) for c in range(NQ)] for r in range(NQ)]
        ws = [o.astype(BF16) for o in _strassen_side(blk, LV, False)]
        for c0 in range(0, FQ, CH):
            ms = []
            for k in range(7 ** LV):
                ms.append(_dot_nt(Z2[slot, k, c0:c0 + CH, :], ws[k]))
                if k % YK == YK - 1:
                    yield
            for r, row in enumerate(_strassen_out(ms, LV)):
                f0 = r * FQ + c0
                z1 = _gelu(_dot(win[f0:f0 + CH, :], xn))
                Hs[f0:f0 + CH, :] = (z1 * (jnp.concatenate(row, axis=1) + b)).astype(BF16)
                yield
        store(cols, x + _dot(wout[...], Hs[...]))

    def transpose_win(j):
        wc = pl.ds(pl.multiple_of(j * WC, 128), WC)
        win[wc, :] = win_raw[:, wc].T

    def a1(i):
        yield from layer_a(xin[:, cols_of(i)].astype(F32), i, cols_of(i))

    def store_y(cols, v):
        Y[...] = v

    def af2(i):
        x = Y[...]
        yield from f_tail(jnp.maximum(i - 1, 0), 1)
        yield from layer_a(x, i, cols_of(i))
        yield from b_front(i, 1)

    with jax.named_scope('loop0'):
        zero_halo()
        Zf[...] = jnp.zeros((FH, BM), F32)
        _interleave(a1(0))
        for j in reversed(range(NWC // 2, NWC)):
            win_copy(j).wait()
            transpose_win(j)

    def loop1(i, _):
        @pl.when(i <= NWC // 2)
        def _():
            win_copy(NWC // 2 - i).wait()
        _interleave(a1(i), seq(f_tail(jnp.maximum(i - 2, 0), 0), b_front(i - 1, 0)))
        transpose_win(jnp.maximum(NWC // 2 - i, 0))

    with jax.named_scope('loop1'):
        jax.lax.fori_loop(1, NB, loop1, None)
    with jax.named_scope('loop1b'):
        cps[3].wait()
        cps[4].wait()
        cps[5].wait()
        zero_halo()
        _interleave(seq(f_tail(NB - 2, 0), b_front(NB - 1, 0), f_tail(NB - 1, 0)))
        _interleave(b_back(0, 0, store_y))

    def loop2(i, _):
        _interleave(af2(i - 1), b_back(i, 0, store_y))

    with jax.named_scope('loop2'):
        jax.lax.fori_loop(1, NB, loop2, None)
    with jax.named_scope('loop2b'):
        _interleave(seq(af2(NB - 1), f_tail(NB - 1, 1)))

    def out_copy(i):
        return pltpu.make_async_copy(obuf.at[:, cols_of(i)], o_hbm.at[:, cols_of(i)], osem.at[i])

    def store_o(cols, v):
        obuf[:, cols] = v.astype(BF16)

    def loop3(i, _):
        _interleave(b_back(i, 1, store_o))
        out_copy(i).start()

    with jax.named_scope('loop3'):
        jax.lax.fori_loop(0, NB, loop3, None)
    for i in range(NB):
        out_copy(i).wait()


@jax.jit
def pallas_interleave_layers__sliding_local_dilated__mixer_gmlp__prompt_kernel(
    A_x, A_wqkv, A_wo, B_x, B_w_in, B_w_sp, B_b_sp, B_w_out,
):
    del B_x
    vm = pltpu.VMEM
    hbm = pl.BlockSpec(memory_space=pltpu.MemorySpace.HBM)
    out = pl.pallas_call(
        _kernel,
        in_specs=[hbm] * 7,
        out_specs=hbm,
        out_shape=jax.ShapeDtypeStruct((D, S), BF16),
        scratch_shapes=[
            vm((D, S), BF16), vm((D, 3 * D), BF16), vm((D, D), BF16),
            vm((5, 3 * D, 128), F32), vm((1792, D), BF16), vm((D, 640), BF16),
            vm((D, 2 * FH), BF16), vm((2 * FH, D), BF16),
            vm((S, S), BF16), vm((1, S), BF16), vm((D, FH), BF16),
            vm((D, S), F32), vm((D, BM), F32), vm((2, D, S), BF16),
            vm((2, 7 ** LV, FQ, SQ), BF16),
            vm((5, HALO + BM, 128), F32), vm((5, HALO + BM, 128), F32),
            vm((BM, 640), BF16), vm((FH, BM), F32), vm((FH, BM), BF16), vm((D, S), BF16),
            pltpu.SemaphoreType.DMA((6,)), pltpu.SemaphoreType.DMA((NWC,)),
            pltpu.SemaphoreType.DMA((NB,)),
        ],
        compiler_params=pltpu.CompilerParams(vmem_limit_bytes=126 * 1024 * 1024),
    )(A_x.reshape(S, D).T, A_wqkv, A_wo, B_w_in, B_w_sp,
      B_b_sp.reshape(1, S), B_w_out.T)
    return out.T.reshape(1, S, D)
```

```python
import math

import jax
import jax.numpy as jnp
import jax.experimental.pallas as pl
import jax.experimental.pallas.tpu as pltpu

S, D, H, DH, W, DIL = 2048, 576, 32, 18, 8, 2
FH = 2304
BM = 256
NB = S // BM
HALO = 16
CH = 576
LV = 1
CF = 384
YK = 1
NQ = 2 ** LV
FQ, BQ, SQ = FH // NQ, BM // NQ, S // NQ
NWC = min(NB, 6) if NB != 4 else 4
WC = 2 * FH // NWC
EPS = 1e-5
F32, BF16 = jnp.float32, jnp.bfloat16


def _dot(a, b):
    return jnp.dot(a, b, preferred_element_type=F32)


def _dot_nt(a, b):
    return jax.lax.dot_general(a, b, (((1,), (1,)), ((), ())), preferred_element_type=F32)


def _ln(x):
    m = jnp.mean(x, axis=0, keepdims=True)
    c = x - m
    v = jnp.mean(c * c, axis=0, keepdims=True)
    return c * jax.lax.rsqrt(v + EPS)


def _gelu(x):
    c0 = math.sqrt(2.0 / math.pi)
    u = x * (c0 + (c0 * 0.044715) * (x * x))
    hx = 0.5 * x
    return hx + hx * jnp.tanh(u)


def _strassen_side(blk, lv, left):
    if lv == 0:
        return [blk[0][0]]
    h = len(blk) // 2
    a11, a12, a21, a22 = (
        [row[c:c + h] for row in blk[r:r + h]] for r in (0, h) for c in (0, h))
    if left:
        ops = [_add(a11, a22), _add(a21, a22), a11, a22, _add(a11, a12),
               _sub(a21, a11), _sub(a12, a22)]
    else:
        ops = [_add(a11, a22), a11, _sub(a12, a22), _sub(a21, a11), a22,
               _add(a11, a12), _add(a21, a22)]
    return [o for m in ops for o in _strassen_side(m, lv - 1, left)]


def _strassen_out(ms, lv):
    if lv == 0:
        return [[ms[0]]]
    n = len(ms) // 7
    m1, m2, m3, m4, m5, m6, m7 = (
        _strassen_out(ms[k * n:(k + 1) * n], lv - 1) for k in range(7))
    c11 = _add(_sub(_add(m1, m4), m5), m7)
    c22 = _add(_add(_sub(m1, m2), m3), m6)
    top = [l + r for l, r in zip(c11, _add(m3, m5))]
    return top + [l + r for l, r in zip(_add(m2, m4), c22)]


def _add(a, b):
    return [[x + y for x, y in zip(r, t)] for r, t in zip(a, b)]


def _sub(a, b):
    return [[x - y for x, y in zip(r, t)] for r, t in zip(a, b)]


def _interleave(*gens):
    gens = list(gens)
    while gens:
        for g in list(gens):
            if next(g, _kernel) is _kernel:
                gens.remove(g)


def _kernel(x_hbm, wqkv_hbm, wo_hbm, win_hbm, wsp_hbm, b_hbm, wout_hbm, o_hbm,
            xin, wqkv_raw, wo_raw, T, wqkv, wo, win_raw, win, wsp, bsp, wout,
            X, Y, XN0, XN1, Z0, Z1, K, V, Os, Zf, Hs, obuf, sems, wsem, osem):
    XN, Z2 = (XN0, XN1), (Z0, Z1)

    def win_copy(j):
        cols = pl.ds(pl.multiple_of(j * WC, 128), WC)
        return pltpu.make_async_copy(win_hbm.at[:, cols], win_raw.at[:, cols], wsem.at[j])

    cps = [
        pltpu.make_async_copy(wqkv_hbm, wqkv_raw, sems.at[0]),
        pltpu.make_async_copy(x_hbm, xin, sems.at[1]),
        pltpu.make_async_copy(wo_hbm, wo_raw, sems.at[2]),
        pltpu.make_async_copy(b_hbm, bsp, sems.at[3]),
        pltpu.make_async_copy(wout_hbm, wout, sems.at[4]),
        pltpu.make_async_copy(wsp_hbm, wsp, sems.at[5]),
    ]
    for c in cps[:3]:
        c.start()

    cps[0].wait()
    for j in range(5):
        n = min(128, D - j * 128)
        T[j, :, 0:n] = wqkv_raw[j * 128:j * 128 + n, :].astype(F32).T

    def gather(base, d, n):
        return [T[j, pl.ds(base + d, H, stride=DH), 0:n[j]] for j in range(5)]

    for part, dst in ((0, 0), (1, 640), (2, 1152)):
        for d in range(DH):
            r = dst + d * H if (part != 1 or d < 16) else 576 + (d - 16) * H
            wqkv[r:r + H, :] = jnp.concatenate(
                gather(part * D, d, (128, 128, 128, 128, 64)), axis=1).astype(BF16)
    wqkv[1728:1792, :] = jnp.zeros((64, D), BF16)
    cps[2].wait()
    for j in range(5):
        n = min(128, D - j * 128)
        T[j, 0:D, 0:n] = wo_raw[:, j * 128:j * 128 + n].astype(F32)
    for t in range(5):
        blk = [jnp.concatenate(gather(0, d, (128, 128, 128, 128, 64)), axis=1)
               if d < DH else jnp.zeros((H, D), F32) for d in range(4 * t, 4 * t + 4)]
        wo[:, t * 128:(t + 1) * 128] = jnp.concatenate(blk, axis=0).T.astype(BF16)
    cps[1].wait()
    for j in reversed(range(NWC)):
        win_copy(j).start()
    for c in cps[3:]:
        c.start()

    qscale = DH ** -0.5 * math.log2(math.e)
    lane = jax.lax.broadcasted_iota(jnp.int32, (BM, 128), 1)

    def zero_halo():
        K[:, 0:HALO, :] = jnp.zeros((5, HALO, 128), F32)
        V[:, 0:HALO, :] = jnp.zeros((5, HALO, 128), F32)

    def layer_a(x, i, cols, slot):
        xn = _ln(x).T.astype(BF16)
        parts = []
        for n0, n1 in ((0, 640), (640, 1152), (1152, 1792)):
            yield
            parts.append(_dot_nt(xn, wqkv[n0:n1, :]))
        qkv = jnp.concatenate(parts, axis=1)
        yield
        t = qkv[:, 512:640]
        q = [qkv[:, j * 128:(j + 1) * 128] * qscale for j in range(4)]
        q.append(jnp.where(lane < 64, t * qscale, 0.0))
        for j in range(4):
            K[j, HALO:, :] = qkv[:, 640 + j * 128:768 + j * 128]
        K[4, HALO:, :] = pltpu.roll(t, 64, 1)
        for j in range(5):
            V[j, HALO:, :] = qkv[:, 1152 + j * 128:1280 + j * 128]
        R = 16
        for r0 in range(0, BM, R):
            lg = []
            for w in range(W):
                s = HALO + r0 - DIL * w
                a = q[0][r0:r0 + R] * K[0, s:s + R, :]
                for j in range(1, 5):
                    a = a + q[j][r0:r0 + R] * K[j, s:s + R, :]
                a = a + pltpu.roll(a, 64, 1)
                a = a + pltpu.roll(a, 32, 1)
                if r0 < DIL * w:
                    row = jax.lax.broadcasted_iota(jnp.int32, (R, 128), 0) + (i * BM + r0)
                    a = jnp.where(row >= DIL * w, a, -1e9)
                lg.append(a)
            m = lg[0]
            for w in range(1, W):
                m = jnp.maximum(m, lg[w])
            p = [jnp.exp2(a - m) for a in lg]
            den = p[0]
            for w in range(1, W):
                den = den + p[w]
            inv = 1.0 / den
            o = []
            for j in range(5):
                a = p[0] * V[j, HALO + r0:HALO + r0 + R, :]
                for w in range(1, W):
                    s = HALO + r0 - DIL * w
                    a = a + p[w] * V[j, s:s + R, :]
                o.append((a * inv).astype(BF16))
            Os[r0:r0 + R, :] = jnp.concatenate(o, axis=1)
            if (r0 + R) % (BM // 4) == 0:
                yield
        for j in range(5):
            K[j, 0:HALO, :] = K[j, BM:BM + HALO, :]
            V[j, 0:HALO, :] = V[j, BM:BM + HALO, :]
        x = x + _dot_nt(wo[...], Os[...])
        X[:, cols] = x
        yield
        XN[slot][:, cols] = _ln(x).astype(BF16)

    def cols_of(i):
        return pl.ds(pl.multiple_of(i * BM, BM), BM)

    def b_front(i, slot):
        cols = cols_of(i)
        xn = XN[slot][:, cols]
        for c0 in range(0, FH, CF):
            yield
            Zf[c0:c0 + CF, :] = _gelu(_dot(win[FH + c0:FH + c0 + CF, :], xn))

    def f_tail(i, slot):
        def total(f):
            acc = f(Zf[0:64, :])
            for r in range(64, FH, 64):
                acc = acc + f(Zf[r:r + 64, :])
            return jnp.sum(acc, axis=0, keepdims=True) * (1.0 / FH)
        m = total(lambda z: z)
        yield
        rs = jax.lax.rsqrt(total(lambda z: (z - m) * (z - m)) + EPS)
        sc = pl.ds(pl.multiple_of(i * BQ, BQ), BQ)
        for r0 in range(0, FQ, 32):
            if r0 % (FQ // 2) == 0:
                yield
            zs = [(Zf[r * FQ + r0:r * FQ + r0 + 32, :] - m) * rs for r in range(NQ)]
            blk = [[z[:, c * BQ:(c + 1) * BQ] for c in range(NQ)] for z in zs]
            for k, o in enumerate(_strassen_side(blk, LV, True)):
                Z2[slot][k, r0:r0 + 32, sc] = o.astype(BF16)

    def seq(*gens):
        for g in gens:
            yield from g

    def b_back(i, slot, store):
        cols = cols_of(i)
        xn = XN[slot][:, cols]
        x = X[:, cols]
        b = bsp[:, cols].astype(F32)
        blk = [[jnp.concatenate(
            [wsp[pl.ds(pl.multiple_of(i * BM + c * BQ, BQ), BQ),
                 n * BM + r * BQ:n * BM + (r + 1) * BQ] for n in range(NB)],
            axis=1).astype(F32) for c in range(NQ)] for r in range(NQ)]
        ws = [o.astype(BF16) for o in _strassen_side(blk, LV, False)]
        for c0 in range(0, FQ, CH):
            ms = []
            for k in range(7 ** LV):
                ms.append(_dot_nt(Z2[slot][k, c0:c0 + CH, :], ws[k]))
                if k % YK == YK - 1:
                    yield
            for r, row in enumerate(_strassen_out(ms, LV)):
                f0 = r * FQ + c0
                z1 = _gelu(_dot(win[f0:f0 + CH, :], xn))
                Hs[f0:f0 + CH, :] = (z1 * (jnp.concatenate(row, axis=1) + b)).astype(BF16)
                yield
        store(cols, x + _dot(wout[...], Hs[...]))

    def transpose_win(j):
        wc = pl.ds(pl.multiple_of(j * WC, 128), WC)
        win[wc, :] = win_raw[:, wc].T

    def a1(i):
        yield from layer_a(xin[:, cols_of(i)].astype(F32), i, cols_of(i), 0)

    def store_y(cols, v):
        Y[...] = v

    def af2(i):
        x = Y[...]
        yield from f_tail(jnp.maximum(i - 1, 0), 1)
        yield from layer_a(x, i, cols_of(i), 1)
        yield from b_front(i, 1)

    with jax.named_scope('loop0'):
        zero_halo()
        Zf[...] = jnp.zeros((FH, BM), F32)
        _interleave(a1(0))
        for j in reversed(range(NWC // 2, NWC)):
            win_copy(j).wait()
            transpose_win(j)

    def loop1(i, _):
        @pl.when(i <= NWC // 2)
        def _():
            win_copy(NWC // 2 - i).wait()
        _interleave(a1(i), seq(f_tail(jnp.maximum(i - 2, 0), 0), b_front(i - 1, 0)))
        transpose_win(jnp.maximum(NWC // 2 - i, 0))

    with jax.named_scope('loop1'):
        jax.lax.fori_loop(1, NB, loop1, None)
    with jax.named_scope('loop1b'):
        cps[3].wait()
        cps[4].wait()
        cps[5].wait()
        zero_halo()
        _interleave(seq(f_tail(NB - 2, 0), b_front(NB - 1, 0), f_tail(NB - 1, 0)))
        _interleave(b_back(0, 0, store_y))

    def loop2(i, _):
        _interleave(af2(i - 1), b_back(i, 0, store_y))

    with jax.named_scope('loop2'):
        jax.lax.fori_loop(1, NB, loop2, None)
    with jax.named_scope('loop2b'):
        _interleave(seq(af2(NB - 1), f_tail(NB - 1, 1)))

    def out_copy(i):
        return pltpu.make_async_copy(obuf.at[:, cols_of(i)], o_hbm.at[:, cols_of(i)], osem.at[i])

    def store_o(cols, v):
        obuf[:, cols] = v.astype(BF16)

    def loop3(i, _):
        _interleave(b_back(i, 1, store_o))
        out_copy(i).start()

    with jax.named_scope('loop3'):
        jax.lax.fori_loop(0, NB, loop3, None)
    for i in range(NB):
        out_copy(i).wait()


@jax.jit
def pallas_interleave_layers__sliding_local_dilated__mixer_gmlp__prompt_kernel(
    A_x, A_wqkv, A_wo, B_x, B_w_in, B_w_sp, B_b_sp, B_w_out,
):
    del B_x
    vm = pltpu.VMEM
    hbm = pl.BlockSpec(memory_space=pltpu.MemorySpace.HBM)
    out = pl.pallas_call(
        _kernel,
        in_specs=[hbm] * 7,
        out_specs=hbm,
        out_shape=jax.ShapeDtypeStruct((D, S), BF16),
        scratch_shapes=[
            vm((D, S), BF16), vm((D, 3 * D), BF16), vm((D, D), BF16),
            vm((5, 3 * D, 128), F32), vm((1792, D), BF16), vm((D, 640), BF16),
            vm((D, 2 * FH), BF16), vm((2 * FH, D), BF16),
            vm((S, S), BF16), vm((1, S), BF16), vm((D, FH), BF16),
            vm((D, S), F32), vm((D, BM), F32), vm((D, S), BF16), vm((D, S), BF16),
            vm((7 ** LV, FQ, SQ), BF16), vm((7 ** LV, FQ, SQ), BF16),
            vm((5, HALO + BM, 128), F32), vm((5, HALO + BM, 128), F32),
            vm((BM, 640), BF16), vm((FH, BM), F32), vm((FH, BM), BF16), vm((D, S), BF16),
            pltpu.SemaphoreType.DMA((6,)), pltpu.SemaphoreType.DMA((NWC,)),
            pltpu.SemaphoreType.DMA((NB,)),
        ],
        compiler_params=pltpu.CompilerParams(vmem_limit_bytes=126 * 1024 * 1024),
    )(A_x.reshape(S, D).T, A_wqkv, A_wo, B_w_in, B_w_sp,
      B_b_sp.reshape(1, S), B_w_out.T)
    return out.T.reshape(1, S, D)
```
